```python
import os as _os
_os.environ.setdefault("JAX_PLATFORMS", "cpu")
import jax
import jax.numpy as jnp

def _softmax(x, axis=-1):
    return jax.nn.softmax(x, axis=axis)
def _gelu(x):
    return jax.nn.gelu(x, approximate=True)
def _silu(x):
    return jax.nn.silu(x)
def _sigmoid(x):
    return jax.nn.sigmoid(x)
def _layernorm(x, axis=-1, eps=1e-5):
    m = jnp.mean(x, axis=axis, keepdims=True)
    v = jnp.var(x, axis=axis, keepdims=True)
    return (x - m) / jnp.sqrt(v + eps)
def _scatter_add(tgt, idx, src, axis=0):
    return tgt.at[idx].add(src)
def _segment_sum(src, seg, n):
    return jax.ops.segment_sum(src, seg, n)
class _Rng:
    def __init__(self, key):
        self._k = key
    def _next(self):
        self._k, sub = jax.random.split(self._k)
        return sub
    def normal(self, shape):
        return jax.random.normal(self._next(), shape, dtype=jnp.bfloat16)
    def randint(self, lo, hi, shape):
        return jax.random.randint(self._next(), shape, lo, hi, dtype=jnp.int32)
    def uniform(self, shape, lo=0.0, hi=1.0):
        return jax.random.uniform(self._next(), shape, jnp.bfloat16, lo, hi)
    def permutation(self, n):
        return jax.random.permutation(self._next(), n)


kernel_name = 'standalone__cross_network_dcn_v2__recsys'

def setup_inputs():
    _rng = _Rng(jax.random.key(int.from_bytes(__import__("os").urandom(4), "little")))
    _w = (lambda a: (lambda t: t.astype(jnp.bfloat16) if jnp.issubdtype(t.dtype, jnp.floating) else t)(jnp.asarray(a)))
    B, F, D, L = 16384, 26, 16, 6
    Din = min(F * D, 512)
    R = max(Din // 4, 2)
    sc = Din ** -0.5
    return {
        "x0": _w((lambda *s: _rng.normal(s) * 0.05)(B, Din)),
        "U":  _w((lambda *s: _rng.normal(s) * 1.6)(L, Din, R) * sc),
        "V":  _w((lambda *s: _rng.normal(s) * 1.6)(L, R, Din) * sc),
        "bs": _w((lambda *s: _rng.normal(s) * 0.05)(L, Din)),
    }

def reference(x0, U, V, bs):
    x = x0
    for l in range(U.shape[0]):
        h = jnp.einsum('rd,bd->br', V[l], x)
        h = jnp.einsum('dr,br->bd', U[l], h)
        x = x0 * (h + bs[l]) + x
    return x
```

```python
import jax
import jax.numpy as jnp
from jax import lax
import jax.experimental.pallas as pl
import jax.experimental.pallas.tpu as pltpu

_F32 = jnp.float32
_BF16 = jnp.bfloat16

_TILE = 128
_LANES = 4
_LAG = 2
_FIRST_GROUPS = 2
_LOOP_GROUPS = 6
_W_STAGES = (1, 3)
_W_WAIT_STEP = 12

_SEM_IN, _SEM_STAGE1, _SEM_STAGE2, _SEM_OUT = range(4)


def _dot(a, b):
    return lax.dot_general(a, b, (((1,), (0,)), ((), ())),
                           preferred_element_type=_F32)


def _cat(xs):
    return xs[0] if len(xs) == 1 else jnp.concatenate(xs, axis=0)


def _dot_rows_descending(load_rows, r0, r1, step, rhs):
    starts = list(range(r0, r1, step))[::-1]
    out = _dot(_cat([load_rows(s, s + step) for s in starts]), rhs)
    return _cat([out[i * step:(i + 1) * step] for i in range(len(starts))][::-1])


def _kernel(x_hbm, u_hbm, v_hbm, b_hbm, o_hbm,
            x_buf, o_buf, u_ref, v_ref, b_ref, va_ref, uw_ref, vb_ref, bt_ref, sem):
    L, D, R = u_ref.shape
    n_groups = x_buf.shape[0]
    group = _LANES * _TILE
    n_loops = (n_groups - _FIRST_GROUPS) // _LOOP_GROUPS
    KA = (D // 128) * 128
    spare = 128 - R
    b2_rows = list(range(KA, D - spare)) + [D - 1]
    row_chunks = [(r, min(r + 128, D)) for r in range(0, D, 128)]

    def column(i, width):
        return i * width if isinstance(i, int) else pl.multiple_of(i * width, width)

    def x_copy(g, s):
        return pltpu.make_async_copy(
            x_hbm.at[:, pl.ds(column(g, group), group)], x_buf.at[g], sem.at[s])

    def o_copy(t):
        return pltpu.make_async_copy(
            o_buf.at[t], o_hbm.at[:, pl.ds(column(t, _TILE), _TILE)], sem.at[_SEM_OUT])

    def w_copies(lo, hi, s):
        return [pltpu.make_async_copy(v_hbm.at[lo:hi], v_ref.at[lo:hi], sem.at[s]),
                pltpu.make_async_copy(u_hbm.at[lo:hi], u_ref.at[lo:hi], sem.at[s])]

    stage0 = w_copies(0, _W_STAGES[0], _SEM_IN) + [
        pltpu.make_async_copy(b_hbm, b_ref, sem.at[_SEM_IN])]
    stage1 = [x_copy(0, _SEM_STAGE1)] + w_copies(*_W_STAGES, _SEM_STAGE1)
    stage2 = w_copies(_W_STAGES[1], L, _SEM_STAGE2) + [
        x_copy(g, _SEM_STAGE2) for g in range(1, _FIRST_GROUPS)]

    def prepare_bias():
        rows = _cat([jnp.zeros((R, D), _F32), b_ref[...].astype(_F32),
                     jnp.zeros((spare - L, D), _F32)])
        bt_ref[...] = rows.T.astype(_BF16)

    def prepare_v(l):
        v = v_ref[l].astype(_F32)
        va_ref[l] = v[:, :KA]
        for j, k in enumerate(b2_rows):
            vb_ref[l, j] = jnp.broadcast_to(v[:, KA:][:, k - KA:k - KA + 1], (R, 128))

    def prepare_u(l):
        lane = lax.broadcasted_iota(jnp.int32, (128, 128), 1)
        row = lax.broadcasted_iota(jnp.int32, (128, 128), 0)
        v_b1 = jnp.concatenate(
            [jnp.zeros((R, R), _F32), v_ref[l].astype(_F32)[:, D - spare:]], axis=1)
        v_b1 = _cat([v_b1, jnp.zeros((spare, 128), _F32)])
        m = jnp.where(lane == 127, (row == R + l).astype(_F32),
                      jnp.where(lane < R, (lane == row).astype(_F32), v_b1)).astype(_BF16)
        for r0, r1 in row_chunks:
            ub = jnp.concatenate([u_ref[l, r0:r1], bt_ref[r0:r1, R:]], axis=1)
            uw_ref[l, r0:r1] = _dot(ub, m).astype(_BF16)

    def block(g0, n, is_first):
        is_last_row = lax.broadcasted_iota(jnp.int32, (spare, _TILE), 0) == spare - 1
        x, hidden = {}, {}

        def x0_rows(t, r0, r1):
            c = (t % _LANES) * _TILE
            return x_buf[g0 + t // _LANES, r0:r1, c:c + _TILE]

        def x_rows(t, l, r0, r1, dtype):
            if l == 0:
                return x0_rows(t, r0, r1).astype(dtype)
            return x[t][r0].astype(dtype)

        def first_matmul(t, l):
            parts = [
                _dot_rows_descending(lambda a, b: va_ref[l, a:b, k:k + 128], 0, R, 8,
                                     x_rows(t, l, k, k + 128, _BF16))
                for k in range(0, KA, 128)]
            x_b = x_rows(t, l, KA, D, _F32)
            acc = None
            for j, k in enumerate(b2_rows):
                term = vb_ref[l, j] * x_b[k - KA:k - KA + 1]
                acc = term if acc is None else acc + term
            for p in parts:
                acc = acc + p
            hidden[t] = _cat(
                [acc, jnp.where(is_last_row, 1.0, x_b[D - spare - KA:])]).astype(_BF16)

        def second_matmul(t, l):
            new = {}
            for r0, r1 in row_chunks:
                hb = _dot_rows_descending(lambda a, b: uw_ref[l, a:b, :], r0, r1, 16,
                                          hidden[t])
                new[r0] = x0_rows(t, r0, r1).astype(_F32) * hb + x_rows(t, l, r0, r1, _F32)
                if l == L - 1:
                    o_buf[g0 * _LANES + t, r0:r1, :] = new[r0].astype(o_buf.dtype)
            x[t] = new
            if l == L - 1:
                o_copy(g0 * _LANES + t).start()

        steps = [(g * _LANES + t, l)
                 for g in range(n) for l in range(L) for t in range(_LANES)]
        for s in range(len(steps) + _LAG):
            if is_first:
                if s == _W_WAIT_STEP:
                    for c in stage2:
                        c.wait()
                    for g in range(n, min(n + _LOOP_GROUPS, n_groups)):
                        x_copy(g, _SEM_IN).start()
                for prepare, delay in ((prepare_v, 0), (prepare_u, 1)):
                    for l in range(_W_STAGES[0], L):
                        ready = _W_WAIT_STEP if l >= _W_STAGES[1] else 0
                        if s == max(_LANES * (l - 1) + delay, ready):
                            prepare(l)
            if s < len(steps):
                first_matmul(*steps[s])
            if s >= _LAG:
                second_matmul(*steps[s - _LAG])

    for c in stage0 + stage1 + stage2:
        c.start()
    for c in stage0:
        c.wait()
    prepare_bias()
    for l in range(_W_STAGES[0]):
        prepare_v(l)
        prepare_u(l)
    for c in stage1:
        c.wait()
    block(0, _FIRST_GROUPS, True)

    def loop_body(i, carry):
        g0 = _FIRST_GROUPS + i * _LOOP_GROUPS
        for g in range(_LOOP_GROUPS):
            x_copy(g0 + g, _SEM_IN).wait()

        @pl.when(i + 1 < n_loops)
        def _():
            for g in range(_LOOP_GROUPS):
                x_copy(g0 + _LOOP_GROUPS + g, _SEM_IN).start()

        block(g0, _LOOP_GROUPS, False)
        return carry

    lax.fori_loop(0, n_loops, loop_body, None)
    pltpu.make_async_copy(o_buf, o_buf, sem.at[_SEM_OUT]).wait()


@jax.jit
def pallas_standalone__cross_network_dcn_v2__recsys_kernel(
    x0: jax.Array,
    U: jax.Array,
    V: jax.Array,
    bs: jax.Array,
):
    B, D = x0.shape
    L, _, R = U.shape
    KA = (D // 128) * 128
    n_groups = B // (_LANES * _TILE)
    assert B % (_LANES * _TILE) == 0
    assert (n_groups - _FIRST_GROUPS) % _LOOP_GROUPS == 0
    out = pl.pallas_call(
        _kernel,
        in_specs=[pl.BlockSpec(memory_space=pl.ANY)] * 4,
        out_specs=pl.BlockSpec(memory_space=pl.ANY),
        out_shape=jax.ShapeDtypeStruct((D, B), x0.dtype),
        scratch_shapes=[
            pltpu.VMEM((n_groups, D, _LANES * _TILE), x0.dtype),
            pltpu.VMEM((n_groups * _LANES, D, _TILE), x0.dtype),
            pltpu.VMEM(U.shape, U.dtype),
            pltpu.VMEM(V.shape, V.dtype),
            pltpu.VMEM(bs.shape, bs.dtype),
            pltpu.VMEM((L, R, KA), _F32),
            pltpu.VMEM((L, D, 128), _BF16),
            pltpu.VMEM((L, D - KA - (128 - R) + 1, R, 128), _F32),
            pltpu.VMEM((D, 128), _BF16),
            pltpu.SemaphoreType.DMA((4,)),
        ],
        compiler_params=pltpu.CompilerParams(
            vmem_limit_bytes=100 * 1024 * 1024, disable_bounds_checks=True),
    )(x0.T, U, V, bs)
    return out.T
```

```python
import jax
import jax.numpy as jnp
from jax import lax
import jax.experimental.pallas as pl
import jax.experimental.pallas.tpu as pltpu

_F32 = jnp.float32
_BF16 = jnp.bfloat16

_TILE = 128
_LANES = 4
_LAG = 2
_FIRST_GROUPS = 5
_LOOP_GROUPS = 9
_SPARE_ROWS = 16


def _dot(a, b):
    return lax.dot_general(a, b, (((1,), (0,)), ((), ())),
                           preferred_element_type=_F32)


def _cat(xs):
    return xs[0] if len(xs) == 1 else jnp.concatenate(xs, axis=0)


def _flip(a, rows):
    return _cat([a[r:r + rows] for r in range(0, a.shape[0], rows)][::-1])


def _kernel(x_hbm, u_hbm, v_hbm, b_hbm, o_hbm,
            x_buf, o_buf, va_ref, vb_ref, uw_ref, b_ref, v_bufs, u_bufs, x_bufs, sem):
    L, D, R = u_hbm.shape
    n_loops = x_buf.shape[0]
    group = _LANES * _TILE
    KA = (D // 128) * 128
    spare = 128 - R
    b2_rows = list(range(KA, D - spare)) + [D - 1]
    row_chunks = [(r, min(r + 128, D)) for r in range(0, D, 128)]

    x_cols = [t * _TILE for t in range(_LANES)] + [g * group for g in range(1, _FIRST_GROUPS)]
    sources = {("x", c): (x_hbm.at[:, pl.ds(c, buf.shape[1])], buf)
               for c, buf in zip(x_cols, x_bufs)}
    for l in range(L):
        sources["v", l] = (v_hbm.at[l], v_bufs[l])
        sources["u", l] = (u_hbm.at[l], u_bufs[l])
    staged = {key: pltpu.make_async_copy(src, buf.at[0:src.shape[0]], sem.at[i])
              for i, (key, (src, buf)) in enumerate(sources.items())}
    b_copy = pltpu.make_async_copy(b_hbm, b_ref, sem.at[len(staged)])
    in_sem, out_sem = sem.at[len(staged) + 1], sem.at[len(staged) + 2]

    def arrived(key, after):
        src, buf = sources[key]
        cols = min(128, buf.shape[1])
        buf[buf.shape[0] - _SPARE_ROWS:, 0:cols] = after[:_SPARE_ROWS, :cols].astype(buf.dtype)
        staged[key].wait()

    def column(i, width, base=0):
        c = base + i * width
        return c if isinstance(i, int) else pl.multiple_of(c, _TILE)

    def x_copy(i):
        width = _LOOP_GROUPS * group
        return pltpu.make_async_copy(
            x_hbm.at[:, pl.ds(column(i, width, _FIRST_GROUPS * group), width)],
            x_buf.at[i, 0:D], in_sem)

    def o_copy(t):
        return pltpu.make_async_copy(
            o_buf.at[t], o_hbm.at[:, pl.ds(column(t, _TILE), _TILE)], out_sem)

    def prepare_v(l):
        v_b = _flip(v_bufs[l][0:R, KA:].astype(_F32), 8)
        for j, k in enumerate(b2_rows):
            vb_ref[l, j] = jnp.broadcast_to(v_b[:, k - KA:k - KA + 1], (R, _TILE))
        va_ref[l] = _flip(v_bufs[l][0:R, :KA].astype(_F32), 8)

    def prepare_u(l):
        v_t = v_bufs[l][0:R, KA:].astype(_F32).T[D - spare - KA:]
        bias = b_ref[...].astype(_F32)[l:l + 1]
        for r0, r1 in row_chunks:
            u = u_bufs[l][r0:r1]
            w_t = lax.dot_general(v_t, u, (((1,), (1,)), ((), ())),
                                  preferred_element_type=_F32)
            is_last = lax.broadcasted_iota(jnp.int32, w_t.shape, 0) == spare - 1
            w_t = jnp.where(is_last, bias[:, r0:r1], w_t)
            w = _cat([jnp.zeros((R, r1 - r0), _F32), w_t]).astype(_BF16).T
            u = jnp.concatenate([u, jnp.zeros((r1 - r0, spare), u.dtype)], axis=1)
            is_u = lax.broadcasted_iota(jnp.int32, (r1 - r0, 128), 1) < R
            uw_ref[l, r0:r1] = _flip(jnp.where(is_u, u, w), 16)

    def block(i):
        first = i is None
        n = _FIRST_GROUPS if first else _LOOP_GROUPS
        tile0 = 0 if first else (_FIRST_GROUPS + i * _LOOP_GROUPS) * _LANES
        is_last_row = lax.broadcasted_iota(jnp.int32, (spare, _TILE), 0) == spare - 1
        x, hidden, done = {}, {}, []

        def x0_rows(t, r0, r1):
            c = t * _TILE
            if not first:
                return x_buf[i, r0:r1, c:c + _TILE]
            start = max(s for s in x_cols if s <= c)
            return sources["x", start][1][r0:r1, c - start:c - start + _TILE]

        def x_rows(t, l, r0, r1):
            return x0_rows(t, r0, r1) if l == 0 else x[t][r0]

        def first_matmul(t, l):
            parts = []
            for k in range(0, KA, 128):
                parts.append(_dot(va_ref[l, :, k:k + 128], x_rows(t, l, k, k + 128)))
                if first and l == 0 and k == 0 and t + 1 < _LANES:
                    arrived(("x", (t + 1) * _TILE), _cat([parts[0][:8]] * 2))
            x_b = x_rows(t, l, KA, D).astype(_F32)
            acc = None
            for j, k in enumerate(b2_rows):
                term = vb_ref[l, j] * x_b[k - KA:k - KA + 1]
                acc = term if acc is None else acc + term
            for p in parts:
                acc = acc + p
            hidden[t] = _cat([_flip(acc, 8),
                              jnp.where(is_last_row, 1.0, x_b[D - spare - KA:])]).astype(_BF16)
            done.append(hidden[t])

        def second_matmul(t, l):
            new = {}
            for r0, r1 in row_chunks:
                hb = _flip(_dot(uw_ref[l, r0:r1], hidden[t]), 16)
                new[r0] = (x0_rows(t, r0, r1).astype(_F32) * hb
                           + x_rows(t, l, r0, r1).astype(_F32))
                if l == L - 1:
                    o_buf[tile0 + t, r0:r1, :] = new[r0].astype(o_buf.dtype)
            x[t] = new
            if l == L - 1:
                o_copy(tile0 + t).start()

        steps = [(g * _LANES + t, l)
                 for g in range(n) for l in range(L) for t in range(_LANES)]
        for s in range(len(steps) + _LAG):
            if first and s == 2 * _LANES:
                x_buf[0, D:, 0:128] = done[s - _LAG][:_SPARE_ROWS]
                x_copy(0).start()
            elif not first and s == 1:
                pl.when(i + 1 < n_loops)(lambda: x_copy(i + 1).start())
            if first and (s + _LAG) % (L * _LANES) == 0 and s + _LAG < len(steps):
                arrived(("x", steps[s + _LAG][0] * _TILE), done[s - _LAG])
            if s < len(steps):
                t, l = steps[s]
                if first and t == 0:
                    if l == 0:
                        prepare_u(0)
                    prepare_v(l)
                first_matmul(t, l)
                if first and t == _LANES - 1 and l + 1 < L:
                    arrived(("v", l + 1), done[s - _LAG])
                if first and t == 0 and l > 0:
                    arrived(("u", l), done[s - _LAG])
                    prepare_u(l)
            if s >= _LAG:
                second_matmul(*steps[s - _LAG])

    staged["v", 0].start()
    b_copy.start()
    staged["u", 0].start()
    for c in x_cols[:_LANES]:
        staged["x", c].start()
    for l in range(1, L):
        staged["v", l].start()
        staged["u", l].start()
    for c in x_cols[_LANES:]:
        staged["x", c].start()

    staged["v", 0].wait()
    b_copy.wait()
    staged["u", 0].wait()
    staged["x", 0].wait()
    block(None)

    def loop_body(i, carry):
        x_copy(i).wait()
        block(i)
        return carry

    lax.fori_loop(0, n_loops, loop_body, None)
    pltpu.make_async_copy(o_hbm, o_hbm, out_sem).wait()


@jax.jit
def pallas_standalone__cross_network_dcn_v2__recsys_kernel(
    x0: jax.Array,
    U: jax.Array,
    V: jax.Array,
    bs: jax.Array,
):
    B, D = x0.shape
    L, _, R = U.shape
    KA = (D // 128) * 128
    group = _LANES * _TILE
    n_loops, rest = divmod(B - _FIRST_GROUPS * group, _LOOP_GROUPS * group)
    assert rest == 0 and n_loops > 0
    x_widths = [_TILE] * _LANES + [group] * (_FIRST_GROUPS - 1)
    out = pl.pallas_call(
        _kernel,
        in_specs=[pl.BlockSpec(memory_space=pl.ANY)] * 4,
        out_specs=pl.BlockSpec(memory_space=pl.ANY),
        out_shape=jax.ShapeDtypeStruct((D, B), x0.dtype),
        scratch_shapes=[
            pltpu.VMEM((n_loops, D + _SPARE_ROWS, _LOOP_GROUPS * group), x0.dtype),
            pltpu.VMEM((B // _TILE, D, _TILE), x0.dtype),
            pltpu.VMEM((L, R, KA), _F32),
            pltpu.VMEM((L, D - KA - (128 - R) + 1, R, _TILE), _F32),
            pltpu.VMEM((L, D, 128), _BF16),
            pltpu.VMEM(bs.shape, bs.dtype),
            [pltpu.VMEM((128, D), V.dtype) for _ in range(L)],
            [pltpu.VMEM((D + _SPARE_ROWS, R), U.dtype) for _ in range(L)],
            [pltpu.VMEM((D + _SPARE_ROWS, w), x0.dtype) for w in x_widths],
            pltpu.SemaphoreType.DMA((len(x_widths) + 2 * L + 3,)),
        ],
        compiler_params=pltpu.CompilerParams(
            vmem_limit_bytes=100 * 1024 * 1024,
            disable_bounds_checks=True,
            disable_semaphore_checks=True,
            flags={"XLA_TPU_RESCHEDULE_DMA_DONES": True}),
    )(x0.T, U, V, bs)
    return out.T
```

```python
import jax
import jax.numpy as jnp
from jax import lax
import jax.experimental.pallas as pl
import jax.experimental.pallas.tpu as pltpu

_F32 = jnp.float32
_BF16 = jnp.bfloat16

_TILE = 128
_LANES = 4
_LAG = 2
_FIRST_GROUPS = 5
_LOOP_GROUPS = 9
_SPARE_ROWS = 16


def _dot(a, b):
    return lax.dot_general(a, b, (((1,), (0,)), ((), ())),
                           preferred_element_type=_F32)


def _cat(xs):
    return xs[0] if len(xs) == 1 else jnp.concatenate(xs, axis=0)


def _flip(a, rows):
    return _cat([a[r:r + rows] for r in range(0, a.shape[0], rows)][::-1])


def _kernel(x_hbm, u_hbm, v_hbm, b_hbm, o_hbm,
            x_buf, o_buf, va_ref, vb_ref, uw_ref, b_ref, v_bufs, u_bufs, x_bufs, sem):
    L, D, R = u_hbm.shape
    n_loops = x_buf.shape[0]
    group = _LANES * _TILE
    KA = (D // 128) * 128
    spare = 128 - R
    b2_rows = list(range(KA, D - spare)) + [D - 1]
    row_chunks = [(r, min(r + 128, D)) for r in range(0, D, 128)]

    x_cols = [t * _TILE for t in range(_LANES)] + [g * group for g in range(1, _FIRST_GROUPS)]
    sources = {("x", c): (x_hbm.at[:, pl.ds(c, buf.shape[1])], buf)
               for c, buf in zip(x_cols, x_bufs)}
    for l in range(L):
        sources["v", l] = (v_hbm.at[l], v_bufs[l])
        sources["u", l] = (u_hbm.at[l], u_bufs[l])
    staged = {key: pltpu.make_async_copy(src, buf.at[0:src.shape[0]], sem.at[i])
              for i, (key, (src, buf)) in enumerate(sources.items())}
    b_copy = pltpu.make_async_copy(b_hbm, b_ref, sem.at[len(staged)])
    in_sem, out_sem = sem.at[len(staged) + 1], sem.at[len(staged) + 2]

    def arrived(key, after):
        buf = sources[key][1]
        cols = min(128, buf.shape[1])
        buf[buf.shape[0] - _SPARE_ROWS:, 0:cols] = after[:_SPARE_ROWS, :cols].astype(buf.dtype)
        staged[key].wait()

    def column(i, width, base=0):
        c = base + i * width
        return c if isinstance(i, int) else pl.multiple_of(c, _TILE)

    def x_copy(i):
        width = _LOOP_GROUPS * group
        return pltpu.make_async_copy(
            x_hbm.at[:, pl.ds(column(i, width, _FIRST_GROUPS * group), width)],
            x_buf.at[i, 0:D], in_sem)

    def o_copy(t):
        return pltpu.make_async_copy(
            o_buf.at[t], o_hbm.at[:, pl.ds(column(t, _TILE), _TILE)], out_sem)

    def prepare_v(l):
        v_b = _flip(v_bufs[l][0:R, KA:].astype(_F32), 8)
        for j, k in enumerate(b2_rows):
            vb_ref[l, j] = jnp.broadcast_to(v_b[:, k - KA:k - KA + 1], (R, _TILE))
        va_ref[l] = _flip(v_bufs[l][0:R, :KA].astype(_F32), 8)

    def prepare_u(l):
        v_t = v_bufs[l][0:R, KA:].astype(_F32).T[D - spare - KA:]
        bias = b_ref[...].astype(_F32)[l:l + 1]
        for r0, r1 in row_chunks:
            u = u_bufs[l][r0:r1]
            w_t = lax.dot_general(v_t, u, (((1,), (1,)), ((), ())),
                                  preferred_element_type=_F32)
            is_last = lax.broadcasted_iota(jnp.int32, w_t.shape, 0) == spare - 1
            w_t = jnp.where(is_last, bias[:, r0:r1], w_t)
            w = _cat([jnp.zeros((R, r1 - r0), _F32), w_t]).astype(_BF16).T
            u = jnp.concatenate([u, jnp.zeros((r1 - r0, spare), u.dtype)], axis=1)
            is_u = lax.broadcasted_iota(jnp.int32, (r1 - r0, 128), 1) < R
            uw_ref[l, r0 // 2:r1 // 2] = pltpu.bitcast(
                _flip(jnp.where(is_u, u, w), 16), jnp.uint32)

    def block(i):
        first = i is None
        n = _FIRST_GROUPS if first else _LOOP_GROUPS
        tile0 = 0 if first else (_FIRST_GROUPS + i * _LOOP_GROUPS) * _LANES
        is_last_row = lax.broadcasted_iota(jnp.int32, (spare, _TILE), 0) == spare - 1
        x, hidden, done = {}, {}, []

        def x0_rows(t, r0, r1):
            c = t * _TILE
            if not first:
                return x_buf[i, r0:r1, c:c + _TILE]
            start = max(s for s in x_cols if s <= c)
            return sources["x", start][1][r0:r1, c - start:c - start + _TILE]

        def x_rows(t, l, r0, r1):
            return x0_rows(t, r0, r1) if l == 0 else x[t][r0]

        def first_matmul(t, l):
            parts = []
            for k in range(0, KA, 128):
                parts.append(_dot(va_ref[l, :, k:k + 128], x_rows(t, l, k, k + 128)))
                if first and l == 0 and k == 0 and t + 1 < _LANES:
                    arrived(("x", (t + 1) * _TILE), _cat([parts[0][:8]] * 2))
            x_b = x_rows(t, l, KA, D).astype(_F32)
            acc = None
            for j, k in enumerate(b2_rows):
                term = vb_ref[l, j] * x_b[k - KA:k - KA + 1]
                acc = term if acc is None else acc + term
            for p in parts:
                acc = acc + p
            hidden[t] = _cat([_flip(acc, 8),
                              jnp.where(is_last_row, 1.0, x_b[D - spare - KA:])]).astype(_BF16)
            done.append(hidden[t])

        def second_matmul(t, l):
            new = {}
            for r0, r1 in row_chunks:
                uw = pltpu.bitcast(uw_ref[l, r0 // 2:r1 // 2], _BF16)
                hb = _flip(_dot(uw, hidden[t]), 16)
                new[r0] = (x0_rows(t, r0, r1).astype(_F32) * hb
                           + x_rows(t, l, r0, r1).astype(_F32))
                if l == L - 1:
                    o_buf[tile0 + t, r0:r1, :] = new[r0].astype(o_buf.dtype)
            x[t] = new
            if l == L - 1:
                o_copy(tile0 + t).start()

        steps = [(g * _LANES + t, l)
                 for g in range(n) for l in range(L) for t in range(_LANES)]
        for s in range(len(steps) + _LAG):
            if first and s == 2 * _LANES:
                x_buf[0, D:, 0:128] = done[s - _LAG][:_SPARE_ROWS]
                x_copy(0).start()
            elif not first and s == 1:
                pl.when(i + 1 < n_loops)(lambda: x_copy(i + 1).start())
            if first and (s + _LAG) % (L * _LANES) == 0 and s + _LAG < len(steps):
                arrived(("x", steps[s + _LAG][0] * _TILE), done[s - _LAG])
            if s < len(steps):
                t, l = steps[s]
                if first and t == 0:
                    if l == 0:
                        prepare_u(0)
                    prepare_v(l)
                first_matmul(t, l)
                if first and t == _LANES - 1 and l + 1 < L:
                    arrived(("v", l + 1), done[s - _LAG])
                if first and t == 0 and l > 0:
                    arrived(("u", l), done[s - _LAG])
                    prepare_u(l)
            if s >= _LAG:
                second_matmul(*steps[s - _LAG])

    staged["v", 0].start()
    b_copy.start()
    staged["u", 0].start()
    for c in x_cols[:_LANES]:
        staged["x", c].start()
    for l in range(1, L):
        staged["v", l].start()
        staged["u", l].start()
    for c in x_cols[_LANES:]:
        staged["x", c].start()

    staged["v", 0].wait()
    b_copy.wait()
    staged["u", 0].wait()
    staged["x", 0].wait()
    block(None)

    def loop_body(i, carry):
        x_copy(i).wait()
        block(i)
        return carry

    lax.fori_loop(0, n_loops, loop_body, None)
    pltpu.make_async_copy(o_hbm, o_hbm, out_sem).wait()


@jax.jit
def pallas_standalone__cross_network_dcn_v2__recsys_kernel(
    x0: jax.Array,
    U: jax.Array,
    V: jax.Array,
    bs: jax.Array,
):
    B, D = x0.shape
    L, _, R = U.shape
    KA = (D // 128) * 128
    group = _LANES * _TILE
    n_loops, rest = divmod(B - _FIRST_GROUPS * group, _LOOP_GROUPS * group)
    assert rest == 0 and n_loops > 0
    x_widths = [_TILE] * _LANES + [group] * (_FIRST_GROUPS - 1)
    out = pl.pallas_call(
        _kernel,
        in_specs=[pl.BlockSpec(memory_space=pl.ANY)] * 4,
        out_specs=pl.BlockSpec(memory_space=pl.ANY),
        out_shape=jax.ShapeDtypeStruct((D, B), x0.dtype),
        scratch_shapes=[
            pltpu.VMEM((n_loops, D + _SPARE_ROWS, _LOOP_GROUPS * group), x0.dtype),
            pltpu.VMEM((B // _TILE, D, _TILE), x0.dtype),
            pltpu.VMEM((L, R, KA), _F32),
            pltpu.VMEM((L, D - KA - (128 - R) + 1, R, _TILE), _F32),
            pltpu.VMEM((L, D // 2, 128), jnp.uint32),
            pltpu.VMEM(bs.shape, bs.dtype),
            [pltpu.VMEM((128, D), V.dtype) for _ in range(L)],
            [pltpu.VMEM((D + _SPARE_ROWS, R), U.dtype) for _ in range(L)],
            [pltpu.VMEM((D + _SPARE_ROWS, w), x0.dtype) for w in x_widths],
            pltpu.SemaphoreType.DMA((len(x_widths) + 2 * L + 3,)),
        ],
        compiler_params=pltpu.CompilerParams(
            vmem_limit_bytes=100 * 1024 * 1024,
            disable_bounds_checks=True,
            disable_semaphore_checks=True,
            flags={"XLA_TPU_RESCHEDULE_DMA_DONES": True}),
    )(x0.T, U, V, bs)
    return out.T
```

```python
import jax
import jax.numpy as jnp
from jax import lax
import jax.experimental.pallas as pl
import jax.experimental.pallas.tpu as pltpu

_F32 = jnp.float32
_BF16 = jnp.bfloat16

_TILE = 128
_LANES = 4
_LAG = 2
_FIRST_GROUPS = 5
_LOOP_GROUPS = 9
_SPARE_ROWS = 16


def _dot(a, b):
    return lax.dot_general(a, b, (((1,), (0,)), ((), ())),
                           preferred_element_type=_F32)


def _cat(xs):
    return xs[0] if len(xs) == 1 else jnp.concatenate(xs, axis=0)


def _sum(xs):
    total = xs[0]
    for x in xs[1:]:
        total = total + x
    return total


def _flip(a, rows):
    return _cat([a[r:r + rows] for r in range(0, a.shape[0], rows)][::-1])


def _kernel(x_hbm, u_hbm, v_hbm, b_hbm, o_hbm,
            x_buf, o_buf, va_ref, vb_ref, uw_ref, b_ref, v_bufs, u_bufs, x_bufs, sem):
    L, D, R = u_hbm.shape
    n_loops = x_buf.shape[0]
    group = _LANES * _TILE
    KA = (D // 128) * 128
    spare = 128 - R
    b2_rows = list(range(KA, D - spare)) + [D - 1]
    row_chunks = [(r, min(r + 128, D)) for r in range(0, D, 128)]

    x_cols = [t * _TILE for t in range(_LANES)] + [g * group for g in range(1, _FIRST_GROUPS)]
    sources = {("x", c): (x_hbm.at[:, pl.ds(c, buf.shape[1])], buf)
               for c, buf in zip(x_cols, x_bufs)}
    for l in range(L):
        sources["v", l] = (v_hbm.at[l], v_bufs[l])
        sources["u", l] = (u_hbm.at[l], u_bufs[l])
    staged = {key: pltpu.make_async_copy(src, buf.at[0:src.shape[0]], sem.at[i])
              for i, (key, (src, buf)) in enumerate(sources.items())}
    b_copy = pltpu.make_async_copy(b_hbm, b_ref, sem.at[len(staged)])
    in_sem, out_sem = sem.at[len(staged) + 1], sem.at[len(staged) + 2]

    def arrived(key, after):
        buf = sources[key][1]
        cols = min(128, buf.shape[1])
        buf[buf.shape[0] - _SPARE_ROWS:, 0:cols] = after[:_SPARE_ROWS, :cols].astype(buf.dtype)
        staged[key].wait()

    def column(i, width, base=0):
        c = base + i * width
        return c if isinstance(i, int) else pl.multiple_of(c, _TILE)

    def x_copy(i):
        width = _LOOP_GROUPS * group
        return pltpu.make_async_copy(
            x_hbm.at[:, pl.ds(column(i, width, _FIRST_GROUPS * group), width)],
            x_buf.at[i, 0:D], in_sem)

    def o_copy(t):
        return pltpu.make_async_copy(
            o_buf.at[t], o_hbm.at[:, pl.ds(column(t, _TILE), _TILE)], out_sem)

    def prepare_v(l):
        v_b = _flip(v_bufs[l][0:R, KA:].astype(_F32), 8)
        for j, k in enumerate(b2_rows):
            vb_ref[l, j] = jnp.broadcast_to(v_b[:, k - KA:k - KA + 1], (R, _TILE))
        va_ref[l] = _flip(v_bufs[l][0:R, :KA].astype(_F32), 8)

    def prepare_u(l):
        v_t = v_bufs[l][0:R, KA:].astype(_F32).T[D - spare - KA:]
        bias = b_ref[...].astype(_F32)[l:l + 1]
        for r0, r1 in row_chunks:
            u = u_bufs[l][r0:r1]
            w_t = lax.dot_general(v_t, u, (((1,), (1,)), ((), ())),
                                  preferred_element_type=_F32)
            is_last = lax.broadcasted_iota(jnp.int32, w_t.shape, 0) == spare - 1
            w_t = jnp.where(is_last, bias[:, r0:r1], w_t)
            w = _cat([jnp.zeros((R, r1 - r0), _F32), w_t]).astype(_BF16).T
            u = jnp.concatenate([u, jnp.zeros((r1 - r0, spare), u.dtype)], axis=1)
            is_u = lax.broadcasted_iota(jnp.int32, (r1 - r0, 128), 1) < R
            uw_ref[l, r0 // 2:r1 // 2] = pltpu.bitcast(
                _flip(jnp.where(is_u, u, w), 16), jnp.uint32)

    def block(i):
        first = i is None
        n = _FIRST_GROUPS if first else _LOOP_GROUPS
        tile0 = 0 if first else (_FIRST_GROUPS + i * _LOOP_GROUPS) * _LANES
        is_last_row = lax.broadcasted_iota(jnp.int32, (spare, _TILE), 0) == spare - 1
        x, hidden, done = {}, {}, []

        def x0_rows(t, r0, r1):
            c = t * _TILE
            if not first:
                return x_buf[i, r0:r1, c:c + _TILE]
            start = max(s for s in x_cols if s <= c)
            return sources["x", start][1][r0:r1, c - start:c - start + _TILE]

        def x_rows(t, l, r0, r1):
            return x0_rows(t, r0, r1) if l == 0 else x[t][r0]

        def first_matmul(t, l):
            parts = []
            for k in range(0, KA, 128):
                parts.append(_dot(va_ref[l, :, k:k + 128], x_rows(t, l, k, k + 128)))
                if first and l == 0 and k == 0 and t + 1 < _LANES:
                    arrived(("x", (t + 1) * _TILE), _cat([parts[0][:8]] * 2))
            x_b = x_rows(t, l, KA, D).astype(_F32)
            terms = [vb_ref[l, j] * x_b[k - KA:k - KA + 1] for j, k in enumerate(b2_rows)]
            m = pl.cdiv(len(terms), len(parts))
            acc = _sum([_sum(terms[j * m:(j + 1) * m] + [p]) for j, p in enumerate(parts)])
            hidden[t] = _cat([_flip(acc, 8),
                              jnp.where(is_last_row, 1.0, x_b[D - spare - KA:])]).astype(_BF16)
            done.append(hidden[t])

        def second_matmul(t, l):
            new = {}
            for r0, r1 in row_chunks:
                uw = pltpu.bitcast(uw_ref[l, r0 // 2:r1 // 2], _BF16)
                hb = _flip(_dot(uw, hidden[t]), 16)
                new[r0] = (x0_rows(t, r0, r1).astype(_F32) * hb
                           + x_rows(t, l, r0, r1).astype(_F32))
                if l == L - 1:
                    o_buf[tile0 + t, r0:r1, :] = new[r0].astype(o_buf.dtype)
            x[t] = new
            if l == L - 1:
                o_copy(tile0 + t).start()

        steps = [(g * _LANES + t, l)
                 for g in range(n) for l in range(L) for t in range(_LANES)]
        for s in range(len(steps) + _LAG):
            if first and s == 2 * _LANES:
                x_buf[0, D:, 0:128] = done[s - _LAG][:_SPARE_ROWS]
                x_copy(0).start()
            elif not first and s == 1:
                pl.when(i + 1 < n_loops)(lambda: x_copy(i + 1).start())
            if first and (s + _LAG) % (L * _LANES) == 0 and s + _LAG < len(steps):
                arrived(("x", steps[s + _LAG][0] * _TILE), done[s - _LAG])
            if s < len(steps):
                t, l = steps[s]
                if first and t == 0:
                    if l == 0:
                        prepare_u(0)
                    prepare_v(l)
                first_matmul(t, l)
                if first and t == _LANES - 1 and l + 1 < L:
                    arrived(("v", l + 1), done[s - _LAG])
                if first and t == 0 and l > 0:
                    arrived(("u", l), done[s - _LAG])
                    prepare_u(l)
            if s >= _LAG:
                second_matmul(*steps[s - _LAG])

    staged["v", 0].start()
    b_copy.start()
    staged["u", 0].start()
    for c in x_cols[:_LANES]:
        staged["x", c].start()
    for l in range(1, L):
        staged["v", l].start()
        staged["u", l].start()
    for c in x_cols[_LANES:]:
        staged["x", c].start()

    staged["v", 0].wait()
    b_copy.wait()
    staged["u", 0].wait()
    staged["x", 0].wait()
    block(None)

    def loop_body(i, carry):
        x_copy(i).wait()
        block(i)
        return carry

    lax.fori_loop(0, n_loops, loop_body, None)
    pltpu.make_async_copy(o_hbm, o_hbm, out_sem).wait()


@jax.jit
def pallas_standalone__cross_network_dcn_v2__recsys_kernel(
    x0: jax.Array,
    U: jax.Array,
    V: jax.Array,
    bs: jax.Array,
):
    B, D = x0.shape
    L, _, R = U.shape
    KA = (D // 128) * 128
    group = _LANES * _TILE
    n_loops, rest = divmod(B - _FIRST_GROUPS * group, _LOOP_GROUPS * group)
    assert rest == 0 and n_loops > 0
    x_widths = [_TILE] * _LANES + [group] * (_FIRST_GROUPS - 1)
    out = pl.pallas_call(
        _kernel,
        in_specs=[pl.BlockSpec(memory_space=pl.ANY)] * 4,
        out_specs=pl.BlockSpec(memory_space=pl.ANY),
        out_shape=jax.ShapeDtypeStruct((D, B), x0.dtype),
        scratch_shapes=[
            pltpu.VMEM((n_loops, D + _SPARE_ROWS, _LOOP_GROUPS * group), x0.dtype),
            pltpu.VMEM((B // _TILE, D, _TILE), x0.dtype),
            pltpu.VMEM((L, R, KA), _F32),
            pltpu.VMEM((L, D - KA - (128 - R) + 1, R, _TILE), _F32),
            pltpu.VMEM((L, D // 2, 128), jnp.uint32),
            pltpu.VMEM(bs.shape, bs.dtype),
            [pltpu.VMEM((128, D), V.dtype) for _ in range(L)],
            [pltpu.VMEM((D + _SPARE_ROWS, R), U.dtype) for _ in range(L)],
            [pltpu.VMEM((D + _SPARE_ROWS, w), x0.dtype) for w in x_widths],
            pltpu.SemaphoreType.DMA((len(x_widths) + 2 * L + 3,)),
        ],
        compiler_params=pltpu.CompilerParams(
            vmem_limit_bytes=100 * 1024 * 1024,
            disable_bounds_checks=True,
            disable_semaphore_checks=True,
            flags={"XLA_TPU_RESCHEDULE_DMA_DONES": True}),
    )(x0.T, U, V, bs)
    return out.T
```
